```python
import jax
import jax.numpy as jnp

def _softmax(x, axis=-1):
    return jax.nn.softmax(x, axis=axis)
def _gelu(x):
    return jax.nn.gelu(x, approximate=True)
def _silu(x):
    return jax.nn.silu(x)
def _sigmoid(x):
    return jax.nn.sigmoid(x)
def _layernorm(x, axis=-1, eps=1e-5):
    m = jnp.mean(x, axis=axis, keepdims=True)
    v = jnp.var(x, axis=axis, keepdims=True)
    return (x - m) / jnp.sqrt(v + eps)
def _scatter_add(tgt, idx, src, axis=0):
    return tgt.at[idx].add(src)
def _segment_sum(src, seg, n):
    return jax.ops.segment_sum(src, seg, n)
class _Rng:
    def __init__(self, key):
        self._k = key
    def _next(self):
        self._k, sub = jax.random.split(self._k)
        return sub
    def normal(self, shape):
        return jax.random.normal(self._next(), shape, dtype=jnp.bfloat16)
    def randint(self, lo, hi, shape):
        return jax.random.randint(self._next(), shape, lo, hi, dtype=jnp.int32)
    def uniform(self, shape, lo=0.0, hi=1.0):
        return jax.random.uniform(self._next(), shape, jnp.bfloat16, lo, hi)
    def permutation(self, n):
        return jax.random.permutation(self._next(), n)


kernel_name = 'recurrent_scan__sliding_block_cached__glu_gated_glu__decode'

def setup_inputs():
    _rng = _Rng(jax.random.key(int.from_bytes(__import__("os").urandom(4), "little")))
    _w = (lambda a: (lambda t: t.astype(jnp.bfloat16) if jnp.issubdtype(t.dtype, jnp.floating) else t)(jnp.asarray(a)))
    def _A_setup():
        B, Sq, D = 1, 1, 576
        Hq, Hkv, Sk, Dh = 32, 16, 65536, 128
        assert Hq % Hkv == 0, (Hq, Hkv)
        return {
            "x": _w((lambda *s: _rng.normal(s) * 0.05)(B, Sq, D)),
            "k_cache": _w((lambda *s: _rng.normal(s) * 0.05)(B, Hkv, Sk, Dh)),
            "v_cache": _w((lambda *s: _rng.normal(s) * 0.05)(B, Hkv, Sk, Dh)),
            "wq": _w((lambda *s: _rng.normal(s) * 0.05)(D, Hq * Dh) * (D ** -0.5)),
            "wo": _w((lambda *s: _rng.normal(s) * 0.05)(Hq * Dh, D) * ((Hq * Dh) ** -0.5)),
        }
    _A_in = _A_setup()

    def _B_setup():
        B, S, D, F = 1, 1, 576, 4608
        return {
            "x": _w((lambda *s: _rng.normal(s) * 0.05)(B, S, D)),
            "w_gate": _w((lambda *s: _rng.normal(s) * 0.05)(D, F)),
            "w_up": _w((lambda *s: _rng.normal(s) * 0.05)(D, F)),
            "w_down": _w((lambda *s: _rng.normal(s) * 0.05)(F, D)),
        }
    _B_in = _B_setup()

    return {
        "A_x": _A_in["x"],
        "A_k_cache": _A_in["k_cache"],
        "A_v_cache": _A_in["v_cache"],
        "A_wq": _A_in["wq"],
        "A_wo": _A_in["wo"],
        "B_x": _B_in["x"],
        "B_w_gate": _B_in["w_gate"],
        "B_w_up": _B_in["w_up"],
        "B_w_down": _B_in["w_down"],
    }

def reference(A_x, A_k_cache, A_v_cache, A_wq, A_wo, B_x, B_w_gate, B_w_up, B_w_down):
    def _A_ref(x, k_cache, v_cache, wq, wo):
        B, Sq, D = x.shape
        Hq, Dh = 32, 128
        Hkv, Sk = k_cache.shape[1], k_cache.shape[2]
        W = min(4096, max(256, Sk // 4))
        rep = Hq // Hkv
        q = (lambda x, *d: x.transpose(*d))((x @ wq).reshape(B, Sq, Hq, Dh), 0, 2, 1, 3)
        k = jnp.repeat(k_cache[:, :, Sk - W:, :], rep, axis=1)
        v = jnp.repeat(v_cache[:, :, Sk - W:, :], rep, axis=1)
        scores = jnp.einsum("bhqd,bhkd->bhqk", q, k) * (Dh ** -0.5)
        p = _softmax(scores, axis=-1)
        o = jnp.einsum("bhqk,bhkd->bhqd", p, v)
        return (lambda x, *d: x.transpose(*d))(o, 0, 2, 1, 3).reshape(B, Sq, Hq * Dh) @ wo

    def _B_ref(x, w_gate, w_up, w_down):
        g = jnp.einsum("bsd,df->bsf", x, w_gate)
        u = jnp.einsum("bsd,df->bsf", x, w_up)
        h = _sigmoid(g) * u
        return jnp.einsum("bsf,fd->bsd", h, w_down)

    x = A_x
    xn = _layernorm(x, axis=-1)
    s = _A_ref(xn, A_k_cache, A_v_cache, A_wq, A_wo)
    g = _silu(_B_ref(xn, B_w_gate, B_w_up, B_w_down))
    return x + s * g
```

```python
import jax
import jax.numpy as jnp
from jax import lax
from jax.experimental import pallas as pl
from jax.experimental.pallas import tpu as pltpu

_BF16 = jnp.bfloat16
_F32 = jnp.float32
_NT = (((1,), (1,)), ((), ()))
_RING = 3
_EPS = 1e-5


def _tail_chunks(d, nq):
    return (
        (0, 384, 0, nq),
        (384, 512, 0, nq),
        (512, d, 0, nq - 1024),
        (512, d, nq - 1024, nq),
    )


@jax.jit
def pallas_recurrent_scan__sliding_block_cached__glu_gated_glu__decode_kernel(
    A_x: jax.Array,
    A_k_cache: jax.Array,
    A_v_cache: jax.Array,
    A_wq: jax.Array,
    A_wo: jax.Array,
    B_x: jax.Array,
    B_w_gate: jax.Array,
    B_w_up: jax.Array,
    B_w_down: jax.Array,
):
    del B_x
    _, _, d = A_x.shape
    _, hkv, sk, dh = A_k_cache.shape
    nq = A_wq.shape[1]
    ff = B_w_gate.shape[1]
    rep = nq // dh // hkv
    win = min(4096, max(256, sk // 4))
    assert rep == 2 and d == 576 and dh == 128
    tail = _tail_chunks(d, nq)
    n_pre = 3
    n_groups = n_pre + hkv + len(tail)
    ring = _RING

    def kernel(x_hbm, k_hbm, v_hbm, wq_hbm, wot_hbm, wg_hbm, wu_hbm, wdt_hbm,
               o_ref,
               x_buf, k_buf, v_buf, wq_buf, wot_buf, wg_buf, wu_buf, wdt_buf,
               o_scr, sems):
        copy = pltpu.make_async_copy

        def head_group(h, sem):
            window = pl.ds(sk - win, win)
            return [copy(k_hbm.at[0, h, window, :], k_buf.at[h], sem),
                    copy(v_hbm.at[0, h, window, :], v_buf.at[h], sem)]

        def tail_group(j, sem):
            r0, r1, c0, c1 = tail[j]
            rows, cols = pl.ds(r0, r1 - r0), pl.ds(c0, c1 - c0)
            return [copy(wot_hbm.at[rows, cols], wot_buf.at[rows, cols], sem)]

        def group(i):
            sem = sems.at[i % ring]
            if i == 0:
                return [copy(wq_hbm, wq_buf, sem), copy(x_hbm, x_buf, sem)]
            if i == 1:
                return [copy(wg_hbm, wg_buf, sem), copy(wu_hbm, wu_buf, sem)]
            if i == 2:
                return [copy(wdt_hbm, wdt_buf, sem)]
            if i < n_pre + hkv:
                return head_group(i - n_pre, sem)
            return tail_group(i - n_pre - hkv, sem)

        def start(copies):
            for c in copies:
                c.start()

        def wait(copies):
            for c in copies:
                c.wait()

        def advance(i):
            wait(group(i))
            if i + ring < n_groups:
                start(group(i + ring))

        for i in range(ring):
            start(group(i))

        advance(0)
        x = x_buf[0].astype(_F32)
        xc = x - jnp.mean(x, axis=-1, keepdims=True)
        var = jnp.mean(xc * xc, axis=-1, keepdims=True)
        xn = (xc / jnp.sqrt(var + _EPS)).astype(_BF16)
        xn8 = jnp.broadcast_to(xn, (8, d))

        advance(1)
        g = jnp.dot(xn8, wg_buf[...], preferred_element_type=_F32)
        u = jnp.dot(xn8, wu_buf[...], preferred_element_type=_F32)
        hid = (jax.nn.sigmoid(g) * u).astype(_BF16)
        advance(2)
        y = lax.dot_general(hid, wdt_buf[...], _NT, preferred_element_type=_F32)
        gate = y * jax.nn.sigmoid(y)

        row = lax.broadcasted_iota(jnp.int32, (8, dh), 0)

        def head(h, carry):
            sem = sems.at[(h + n_pre) % ring]
            wait(head_group(h, sem))

            @pl.when(h + ring < hkv)
            def _():
                start(head_group(h + ring, sem))

            for j in range(ring):
                @pl.when(h == hkv - ring + j)
                def _():
                    start(tail_group(j, sem))

            off = pl.multiple_of(h * (rep * dh), rep * dh)
            qq = jnp.dot(xn8, wq_buf[:, pl.ds(off, rep * dh)],
                         preferred_element_type=_F32)
            q = jnp.where(row == 0, qq[:, :dh], qq[:, dh:]).astype(_BF16)
            s = lax.dot_general(q, k_buf[h], _NT, preferred_element_type=_F32)
            s = s * (dh ** -0.5)
            p = jnp.exp(s - jnp.max(s, axis=-1, keepdims=True))
            denom = jnp.sum(p, axis=-1, keepdims=True)
            o = jnp.dot(p.astype(_BF16), v_buf[h], preferred_element_type=_F32)
            o = o / denom
            o_scr[:, pl.ds(off, dh)] = jnp.broadcast_to(o[0:1], (8, dh)).astype(_BF16)
            o_scr[:, pl.ds(off + dh, dh)] = jnp.broadcast_to(o[1:2], (8, dh)).astype(_BF16)
            return carry

        lax.fori_loop(0, hkv, head, 0)

        partial = {}
        last = {(r0, r1): j for j, (r0, r1, _, _) in enumerate(tail)}
        for j, (r0, r1, c0, c1) in enumerate(tail):
            advance(n_pre + hkv + j)
            so = lax.dot_general(o_scr[:, c0:c1], wot_buf[r0:r1, c0:c1], _NT,
                                 preferred_element_type=_F32)
            if (r0, r1) in partial:
                so = so + partial[(r0, r1)]
            partial[(r0, r1)] = so
            if last[(r0, r1)] == j:
                res = x[:, r0:r1] + (so * gate[:, r0:r1])[0:1]
                o_ref[0, :, r0:r1] = res.astype(_BF16)

    hbm = pl.BlockSpec(memory_space=pl.ANY)
    return pl.pallas_call(
        kernel,
        out_shape=jax.ShapeDtypeStruct(A_x.shape, A_x.dtype),
        in_specs=[hbm] * 8,
        out_specs=pl.BlockSpec(memory_space=pltpu.VMEM),
        scratch_shapes=[
            pltpu.VMEM(A_x.shape, _BF16),
            pltpu.VMEM((hkv, win, dh), _BF16),
            pltpu.VMEM((hkv, win, dh), _BF16),
            pltpu.VMEM((d, nq), _BF16),
            pltpu.VMEM((d, nq), _BF16),
            pltpu.VMEM((d, ff), _BF16),
            pltpu.VMEM((d, ff), _BF16),
            pltpu.VMEM((d, ff), _BF16),
            pltpu.VMEM((8, nq), _BF16),
            pltpu.SemaphoreType.DMA((ring,)),
        ],
        compiler_params=pltpu.CompilerParams(vmem_limit_bytes=96 * 1024 * 1024),
    )(A_x, A_k_cache, A_v_cache, A_wq, A_wo.T, B_w_gate, B_w_up, B_w_down.T)
```

```python
import jax
import jax.numpy as jnp
from jax import lax
from jax.experimental import pallas as pl
from jax.experimental.pallas import tpu as pltpu

_BF16 = jnp.bfloat16
_F32 = jnp.float32
_NT = (((1,), (1,)), ((), ()))
_RING = 4
_EPS = 1e-5


def _tail_chunks(d, nq):
    return (
        (0, 256, 0, nq),
        (256, 384, 0, nq),
        (384, 464, 0, nq),
        (464, 512, 0, nq),
        (512, d, 0, nq - 2560),
        (512, d, nq - 2560, nq - 1024),
        (512, d, nq - 1024, nq),
    )


@jax.jit
def pallas_recurrent_scan__sliding_block_cached__glu_gated_glu__decode_kernel(
    A_x: jax.Array,
    A_k_cache: jax.Array,
    A_v_cache: jax.Array,
    A_wq: jax.Array,
    A_wo: jax.Array,
    B_x: jax.Array,
    B_w_gate: jax.Array,
    B_w_up: jax.Array,
    B_w_down: jax.Array,
):
    del B_x
    _, _, d = A_x.shape
    _, hkv, sk, dh = A_k_cache.shape
    nq = A_wq.shape[1]
    ff = B_w_gate.shape[1]
    rep = nq // dh // hkv
    win = min(4096, max(256, sk // 4))
    assert rep == 2 and d == 576 and dh == 128 and nq == 4096
    tail = _tail_chunks(d, nq)
    n_pre = 3
    n_groups = n_pre + hkv + len(tail)
    ring = _RING

    def kernel(x_hbm, k_hbm, v_hbm, wq_hbm, wot_hbm, wg_hbm, wu_hbm, wdt_hbm,
               out_hbm,
               x_buf, k_buf, v_buf, wq_buf, wot_buf, wg_buf, wu_buf, wdt_buf,
               o_scr, out_buf):
        copy = pltpu.make_async_copy

        def body(sems, out_sem):
            def head_group(h, sem):
                window = pl.ds(sk - win, win)
                return [copy(k_hbm.at[0, h, window, :], k_buf.at[h], sem),
                        copy(v_hbm.at[0, h, window, :], v_buf.at[h], sem)]

            def tail_group(j, sem):
                r0, r1, c0, c1 = tail[j]
                rows, cols = pl.ds(r0, r1 - r0), pl.ds(c0, c1 - c0)
                return [copy(wot_hbm.at[rows, cols], wot_buf.at[rows, cols], sem)]

            def group(i):
                sem = sems.at[i % ring]
                if i == 0:
                    return [copy(wq_hbm, wq_buf, sem), copy(x_hbm, x_buf, sem)]
                if i == 1:
                    return [copy(wg_hbm, wg_buf, sem), copy(wu_hbm, wu_buf, sem)]
                if i == 2:
                    return [copy(wdt_hbm, wdt_buf, sem)]
                if i < n_pre + hkv:
                    return head_group(i - n_pre, sem)
                return tail_group(i - n_pre - hkv, sem)

            def start(copies):
                for c in copies:
                    c.start()

            def wait(copies):
                for c in copies:
                    c.wait()

            def advance(i):
                wait(group(i))
                if i + ring < n_groups:
                    start(group(i + ring))

            for i in range(ring):
                start(group(i))

            advance(0)
            x = x_buf[0].astype(_F32)
            xc = x - jnp.mean(x, axis=-1, keepdims=True)
            var = jnp.mean(xc * xc, axis=-1, keepdims=True)
            xn = (xc / jnp.sqrt(var + _EPS)).astype(_BF16)
            xn8 = jnp.broadcast_to(xn, (8, d))

            advance(1)
            g = jnp.dot(xn8, wg_buf[...], preferred_element_type=_F32)
            u = jnp.dot(xn8, wu_buf[...], preferred_element_type=_F32)
            hid = (jax.nn.sigmoid(g) * u).astype(_BF16)
            advance(2)
            y = lax.dot_general(hid, wdt_buf[...], _NT,
                                preferred_element_type=_F32)
            gate = y * jax.nn.sigmoid(y)

            row = lax.broadcasted_iota(jnp.int32, (8, dh), 0)

            def head(h, carry):
                sem = sems.at[(h + n_pre) % ring]
                wait(head_group(h, sem))

                @pl.when(h + ring < hkv)
                def _():
                    start(head_group(h + ring, sem))

                for j in range(ring):
                    @pl.when(h == hkv - ring + j)
                    def _():
                        start(tail_group(j, sem))

                off = pl.multiple_of(h * (rep * dh), rep * dh)
                qq = jnp.dot(xn8, wq_buf[:, pl.ds(off, rep * dh)],
                             preferred_element_type=_F32)
                q = jnp.where(row == 0, qq[:, :dh], qq[:, dh:]).astype(_BF16)
                s = lax.dot_general(q, k_buf[h], _NT,
                                    preferred_element_type=_F32)
                s = s * (dh ** -0.5)
                p = jnp.exp(s - jnp.max(s, axis=-1, keepdims=True))
                denom = jnp.sum(p, axis=-1, keepdims=True)
                o = jnp.dot(p.astype(_BF16), v_buf[h],
                            preferred_element_type=_F32)
                o = (o / denom).astype(_BF16)
                o_scr[:, pl.ds(off, dh)] = jnp.broadcast_to(o[0:1], (8, dh))
                o_scr[:, pl.ds(off + dh, dh)] = jnp.broadcast_to(o[1:2], (8, dh))
                return carry

            lax.fori_loop(0, hkv, head, 0)

            partial = {}
            last = {(r0, r1): j for j, (r0, r1, _, _) in enumerate(tail)}
            for j, (r0, r1, c0, c1) in enumerate(tail):
                advance(n_pre + hkv + j)
                so = lax.dot_general(o_scr[:, c0:c1], wot_buf[r0:r1, c0:c1],
                                     _NT, preferred_element_type=_F32)
                if (r0, r1) in partial:
                    so = so + partial[(r0, r1)]
                partial[(r0, r1)] = so
                if last[(r0, r1)] == j:
                    res = x[:, r0:r1] + (so * gate[:, r0:r1])[0:1]
                    out_buf[0, :, r0:r1] = res.astype(_BF16)

            write_out = copy(out_buf, out_hbm, out_sem.at[0])
            write_out.start()
            write_out.wait()

        pl.run_scoped(body, pltpu.SemaphoreType.DMA((ring,)),
                      pltpu.SemaphoreType.DMA((1,)))

    hbm = pl.BlockSpec(memory_space=pl.ANY)
    return pl.pallas_call(
        kernel,
        out_shape=jax.ShapeDtypeStruct(A_x.shape, A_x.dtype),
        in_specs=[hbm] * 8,
        out_specs=hbm,
        scratch_shapes=[
            pltpu.VMEM(A_x.shape, _BF16),
            pltpu.VMEM((hkv, win, dh), _BF16),
            pltpu.VMEM((hkv, win, dh), _BF16),
            pltpu.VMEM((d, nq), _BF16),
            pltpu.VMEM((d, nq), _BF16),
            pltpu.VMEM((d, ff), _BF16),
            pltpu.VMEM((d, ff), _BF16),
            pltpu.VMEM((d, ff), _BF16),
            pltpu.VMEM((8, nq), _BF16),
            pltpu.VMEM(A_x.shape, _BF16),
        ],
        compiler_params=pltpu.CompilerParams(vmem_limit_bytes=96 * 1024 * 1024),
    )(A_x, A_k_cache, A_v_cache, A_wq, A_wo.T, B_w_gate, B_w_up, B_w_down.T)
```

```python
import jax
import jax.numpy as jnp
from jax import lax
from jax.experimental import pallas as pl
from jax.experimental.pallas import tpu as pltpu

_BF16 = jnp.bfloat16
_F32 = jnp.float32
_NT = (((1,), (1,)), ((), ()))
_RING = 4
_EPS = 1e-5


def _tail_chunks(d, nq):
    return (
        (0, 256, 0, nq),
        (256, 384, 0, nq),
        (384, 464, 0, nq),
        (464, 512, 0, nq),
        (512, d, 0, nq - 2560),
        (512, d, nq - 2560, nq - 1024),
        (512, d, nq - 1024, nq),
    )


@jax.jit
def pallas_recurrent_scan__sliding_block_cached__glu_gated_glu__decode_kernel(
    A_x: jax.Array,
    A_k_cache: jax.Array,
    A_v_cache: jax.Array,
    A_wq: jax.Array,
    A_wo: jax.Array,
    B_x: jax.Array,
    B_w_gate: jax.Array,
    B_w_up: jax.Array,
    B_w_down: jax.Array,
):
    del B_x
    _, _, d = A_x.shape
    _, hkv, sk, dh = A_k_cache.shape
    nq = A_wq.shape[1]
    ff = B_w_gate.shape[1]
    rep = nq // dh // hkv
    win = min(4096, max(256, sk // 4))
    assert rep == 2 and d == 576 and dh == 128 and nq == 4096
    tail = _tail_chunks(d, nq)
    n_pre = 3
    n_groups = n_pre + hkv + len(tail)
    ring = _RING
    split = 512

    def kernel(x_hbm, k_hbm, v_hbm, wq_hbm, wot_hbm, wg_hbm, wu_hbm, wdt_hbm,
               out_hbm,
               x_buf, k_buf, v_buf, wq_buf, wot_buf, wg_buf, wu_buf, wdt_buf,
               o_scr, out_buf):
        copy = pltpu.make_async_copy

        def body(sems, out_sems):
            def head_group(h, sem):
                window = pl.ds(sk - win, win)
                return [copy(k_hbm.at[0, h, window, :], k_buf.at[h], sem),
                        copy(v_hbm.at[0, h, window, :], v_buf.at[h], sem)]

            def tail_group(j, sem):
                r0, r1, c0, c1 = tail[j]
                rows, cols = pl.ds(r0, r1 - r0), pl.ds(c0, c1 - c0)
                return [copy(wot_hbm.at[rows, cols], wot_buf.at[rows, cols], sem)]

            def group(i):
                sem = sems.at[i % ring]
                if i == 0:
                    return [copy(wq_hbm, wq_buf, sem), copy(x_hbm, x_buf, sem)]
                if i == 1:
                    return [copy(wg_hbm, wg_buf, sem), copy(wu_hbm, wu_buf, sem)]
                if i == 2:
                    return [copy(wdt_hbm, wdt_buf, sem)]
                if i < n_pre + hkv:
                    return head_group(i - n_pre, sem)
                return tail_group(i - n_pre - hkv, sem)

            def write_out(part):
                cols = pl.ds(0, split) if part == 0 else pl.ds(split, d - split)
                return copy(out_buf.at[:, :, cols], out_hbm.at[:, :, cols],
                            out_sems.at[part])

            def start(copies):
                for c in copies:
                    c.start()

            def wait(copies):
                for c in copies:
                    c.wait()

            def advance(i):
                wait(group(i))
                if i + ring < n_groups:
                    start(group(i + ring))

            for i in range(ring):
                start(group(i))

            advance(0)
            x = x_buf[0].astype(_F32)
            xc = x - jnp.mean(x, axis=-1, keepdims=True)
            var = jnp.mean(xc * xc, axis=-1, keepdims=True)
            xn = (xc / jnp.sqrt(var + _EPS)).astype(_BF16)
            xn8 = jnp.broadcast_to(xn, (8, d))

            advance(1)
            g = jnp.dot(xn8, wg_buf[...], preferred_element_type=_F32)
            u = jnp.dot(xn8, wu_buf[...], preferred_element_type=_F32)
            hid = (jax.nn.sigmoid(g) * u).astype(_BF16)
            advance(2)
            y = lax.dot_general(hid, wdt_buf[...], _NT,
                                preferred_element_type=_F32)
            gate = y * jax.nn.sigmoid(y)

            row = lax.broadcasted_iota(jnp.int32, (8, dh), 0)

            def head(h, carry):
                sem = sems.at[(h + n_pre) % ring]
                wait(head_group(h, sem))

                @pl.when(h + ring < hkv)
                def _():
                    start(head_group(h + ring, sem))

                for j in range(ring):
                    @pl.when(h == hkv - ring + j)
                    def _():
                        start(tail_group(j, sem))

                off = pl.multiple_of(h * (rep * dh), rep * dh)
                qq = jnp.dot(xn8, wq_buf[:, pl.ds(off, rep * dh)],
                             preferred_element_type=_F32)
                q = jnp.where(row == 0, qq[:, :dh], qq[:, dh:]).astype(_BF16)
                s = lax.dot_general(q, k_buf[h], _NT,
                                    preferred_element_type=_F32)
                s = s * (dh ** -0.5)
                p = jnp.exp(s - jnp.max(s, axis=-1, keepdims=True))
                denom = jnp.sum(p, axis=-1, keepdims=True)
                o = jnp.dot(p.astype(_BF16), v_buf[h],
                            preferred_element_type=_F32)
                o = (o / denom).astype(_BF16)
                o_scr[:, pl.ds(off, dh)] = jnp.broadcast_to(o[0:1], (8, dh))
                o_scr[:, pl.ds(off + dh, dh)] = jnp.broadcast_to(o[1:2], (8, dh))
                return carry

            lax.fori_loop(0, hkv, head, 0)

            partial = {}
            last = {(r0, r1): j for j, (r0, r1, _, _) in enumerate(tail)}
            for j, (r0, r1, c0, c1) in enumerate(tail):
                advance(n_pre + hkv + j)
                so = lax.dot_general(o_scr[:, c0:c1], wot_buf[r0:r1, c0:c1],
                                     _NT, preferred_element_type=_F32)
                if (r0, r1) in partial:
                    so = so + partial[(r0, r1)]
                partial[(r0, r1)] = so
                if last[(r0, r1)] == j:
                    res = x[:, r0:r1] + (so * gate[:, r0:r1])[0:1]
                    out_buf[0, :, r0:r1] = res.astype(_BF16)
                    if r1 == split:
                        write_out(0).start()
            write_out(1).start()
            write_out(0).wait()
            write_out(1).wait()

        pl.run_scoped(body, pltpu.SemaphoreType.DMA((ring,)),
                      pltpu.SemaphoreType.DMA((2,)))

    hbm = pl.BlockSpec(memory_space=pl.ANY)
    return pl.pallas_call(
        kernel,
        out_shape=jax.ShapeDtypeStruct(A_x.shape, A_x.dtype),
        in_specs=[hbm] * 8,
        out_specs=hbm,
        scratch_shapes=[
            pltpu.VMEM(A_x.shape, _BF16),
            pltpu.VMEM((hkv, win, dh), _BF16),
            pltpu.VMEM((hkv, win, dh), _BF16),
            pltpu.VMEM((d, nq), _BF16),
            pltpu.VMEM((d, nq), _BF16),
            pltpu.VMEM((d, ff), _BF16),
            pltpu.VMEM((d, ff), _BF16),
            pltpu.VMEM((d, ff), _BF16),
            pltpu.VMEM((8, nq), _BF16),
            pltpu.VMEM(A_x.shape, _BF16),
        ],
        compiler_params=pltpu.CompilerParams(vmem_limit_bytes=96 * 1024 * 1024),
    )(A_x, A_k_cache, A_v_cache, A_wq, A_wo.T, B_w_gate, B_w_up, B_w_down.T)
```
